```python
import jax
import jax.numpy as jnp

def _softmax(x, axis=-1):
    return jax.nn.softmax(x, axis=axis)
def _gelu(x):
    return jax.nn.gelu(x, approximate=True)
def _silu(x):
    return jax.nn.silu(x)
def _sigmoid(x):
    return jax.nn.sigmoid(x)
def _layernorm(x, axis=-1, eps=1e-5):
    m = jnp.mean(x, axis=axis, keepdims=True)
    v = jnp.var(x, axis=axis, keepdims=True)
    return (x - m) / jnp.sqrt(v + eps)
def _scatter_add(tgt, idx, src, axis=0):
    return tgt.at[idx].add(src)
def _segment_sum(src, seg, n):
    return jax.ops.segment_sum(src, seg, n)
class _Rng:
    def __init__(self, key):
        self._k = key
    def _next(self):
        self._k, sub = jax.random.split(self._k)
        return sub
    def normal(self, shape):
        return jax.random.normal(self._next(), shape, dtype=jnp.bfloat16)
    def randint(self, lo, hi, shape):
        return jax.random.randint(self._next(), shape, lo, hi, dtype=jnp.int32)
    def uniform(self, shape, lo=0.0, hi=1.0):
        return jax.random.uniform(self._next(), shape, jnp.bfloat16, lo, hi)
    def permutation(self, n):
        return jax.random.permutation(self._next(), n)


kernel_name = 'recurrent_scan__compressed_kv_cla__dense_activation_gelu__decode'

def setup_inputs():
    _rng = _Rng(jax.random.key(int.from_bytes(__import__("os").urandom(4), "little")))
    _w = (lambda a: (lambda t: t.astype(jnp.bfloat16) if jnp.issubdtype(t.dtype, jnp.floating) else t)(jnp.asarray(a)))
    def _A_setup():
        B, H, Sq, Sk, D, M = 2, 32, 1, 16384, 128, 512
        Dc = 4 * D
        return {
            "x": _w((lambda *s: _rng.normal(s) * 0.05)(B, Sq, M)),
            "c_kv": _w((lambda *s: _rng.normal(s) * 0.05)(B, Sk, Dc)),
            "w_q": _w((lambda *s: _rng.normal(s) * 0.05)(M, H, D) * (M ** -0.5)),
            "w_uk": _w((lambda *s: _rng.normal(s) * 0.05)(Dc, H, D) * (Dc ** -0.5)),
            "w_uv": _w((lambda *s: _rng.normal(s) * 0.05)(Dc, H, D) * (Dc ** -0.5)),
            "w_o": _w((lambda *s: _rng.normal(s) * 0.05)(H, D, M) * ((H * D) ** -0.5)),
        }
    _A_in = _A_setup()

    def _B_setup():
        B, S, D, F = 2, 1, 512, 1792
        return {
            "x": _w((lambda *s: _rng.normal(s) * 0.05)(B, S, D)),
            "w1": _w((lambda *s: _rng.normal(s) * 0.05)(D, F) * (D ** -0.5)),
            "b1": _w((lambda *s: _rng.normal(s) * 0.05)(F) * 0.01),
            "w2": _w((lambda *s: _rng.normal(s) * 0.05)(F, D) * (F ** -0.5)),
            "b2": _w((lambda *s: _rng.normal(s) * 0.05)(D) * 0.01),
        }
    _B_in = _B_setup()

    return {
        "A_x": _A_in["x"],
        "A_c_kv": _A_in["c_kv"],
        "A_w_q": _A_in["w_q"],
        "A_w_uk": _A_in["w_uk"],
        "A_w_uv": _A_in["w_uv"],
        "A_w_o": _A_in["w_o"],
        "B_x": _B_in["x"],
        "B_w1": _B_in["w1"],
        "B_b1": _B_in["b1"],
        "B_w2": _B_in["w2"],
        "B_b2": _B_in["b2"],
    }

def reference(A_x, A_c_kv, A_w_q, A_w_uk, A_w_uv, A_w_o, B_x, B_w1, B_b1, B_w2, B_b2):
    def _A_ref(x, c_kv, w_q, w_uk, w_uv, w_o):
        B, Sq, M = x.shape[0], x.shape[1], x.shape[2]
        Sk = c_kv.shape[1]
        H, D = w_q.shape[1], w_q.shape[2]
        q = jnp.einsum("bqm,mhd->bhqd", x, w_q)
        k = jnp.einsum("bkc,chd->bhkd", c_kv, w_uk)
        v = jnp.einsum("bkc,chd->bhkd", c_kv, w_uv)
        scores = jnp.einsum("bhqd,bhkd->bhqk", q, k) * (D ** -0.5)
        off = Sk - Sq
        qi = jnp.arange(Sq)[:, None]
        kj = jnp.arange(Sk)[None, :]
        cmask = kj <= (qi + off)
        scores = jnp.where(cmask[None, None], scores, -1e9)
        p = _softmax(scores, axis=-1)
        ctx = jnp.einsum("bhqk,bhkd->bhqd", p, v)
        return jnp.einsum("bhqd,hdm->bqm", ctx, w_o)

    def _B_ref(x, w1, b1, w2, b2):
        h = jnp.einsum("bsd,df->bsf", x, w1) + b1
        h = _gelu(h)
        return jnp.einsum("bsf,fd->bsd", h, w2) + b2

    x = A_x
    xn = _layernorm(x, axis=-1)
    s = _A_ref(xn, A_c_kv, A_w_q, A_w_uk, A_w_uv, A_w_o)
    g = _silu(_B_ref(xn, B_w1, B_b1, B_w2, B_b2))
    return x + s * g
```

```python
import jax
import jax.numpy as jnp
from jax import lax
import jax.experimental.pallas as pl
import jax.experimental.pallas.tpu as pltpu

B, H, D, M, DC, SK, F = 2, 32, 128, 512, 512, 16384, 1792
KT = 1024
CKV1_SPLITS = (0, 8192, 12288, 14336, 16384)
WO_SPLITS = (0, 16, 24, 28, 30, 31, 32)
NT = (((1,), (1,)), ((), ()))
F32, BF16 = jnp.float32, jnp.bfloat16


def _kernel(x_hbm, ckv_hbm, wq_hbm, wuk_hbm, wuv_hbm, wo_hbm, w1_hbm, b1_hbm, w2_hbm, b2_hbm,
            o_hbm,
            x_v, b1_v, b2_v, wq_v, wuk_v, wuv_v, wo_v, w1_v, w2_v, ckv_v,
            e0_v, lhs_v, lo_v, out_v, sems):
    copies = [
        (x_hbm, x_v), (wq_hbm, wq_v), (wuk_hbm, wuk_v), (ckv_hbm.at[0], ckv_v.at[0]),
    ]
    I_X, I_WQ, I_WUK, I_C0 = range(4)
    I_C1 = len(copies)
    for lo, hi in zip(CKV1_SPLITS[:-1], CKV1_SPLITS[1:]):
        copies.append((ckv_hbm.at[1, pl.ds(lo, hi - lo)], ckv_v.at[1, pl.ds(lo, hi - lo)]))
    I_WUV = len(copies)
    copies += [(wuv_hbm, wuv_v), (b1_hbm, b1_v), (b2_hbm, b2_v), (w1_hbm, w1_v), (w2_hbm, w2_v)]
    I_B1, I_B2, I_W1, I_W2 = I_WUV + 1, I_WUV + 2, I_WUV + 3, I_WUV + 4
    I_WO = len(copies)
    for lo, hi in zip(WO_SPLITS[:-1], WO_SPLITS[1:]):
        copies.append((wo_hbm.at[pl.ds(lo, hi - lo)], wo_v.at[pl.ds(lo, hi - lo)]))
    I_OUT = len(copies)
    copies.append((out_v, o_hbm))

    def dma(i):
        return pltpu.make_async_copy(copies[i][0], copies[i][1], sems.at[i])

    for i in range(I_OUT):
        dma(i).start()

    def gen_e0(t, c):
        r = lax.broadcasted_iota(jnp.int32, (128, 128), 1) + t * 128
        m = lax.broadcasted_iota(jnp.int32, (128, 128), 0)
        e0_v[:, pl.ds(pl.multiple_of(t * 128, 128), 128)] = jnp.where((r >> 5) == m, 1.0, 0.0).astype(BF16)
        return c
    lax.fori_loop(0, 32, gen_e0, 0)

    row = lax.broadcasted_iota(jnp.int32, (64, 128), 0)
    lane = lax.broadcasted_iota(jnp.int32, (64, 128), 1)
    diag = (row & 31) == (lane & 31)

    def mask_diag(v):
        parts = [jnp.where(diag, v[:, t * 128:(t + 1) * 128], 0.0) for t in range(v.shape[1] // 128)]
        return jnp.concatenate(parts, axis=1).astype(BF16)

    def expand_matmul(w_v):
        def body(j, acc):
            xr = jnp.dot(lhs_v[j], e0_v[...], preferred_element_type=F32)
            w = w_v[pl.ds(pl.multiple_of(j * 4096, 4096), 4096), :]
            return acc + jnp.dot(mask_diag(xr), w, preferred_element_type=F32)
        return lax.fori_loop(0, 4, body, jnp.zeros((64, 128), F32))

    dma(I_X).wait()
    xs, xns = [], []
    for b in range(B):
        xb = x_v[b].astype(F32)
        mu = jnp.mean(xb, axis=-1, keepdims=True)
        xc = xb - mu
        var = jnp.mean(xc * xc, axis=-1, keepdims=True)
        xs.append(xb)
        xns.append(xc / jnp.sqrt(var + 1e-5))
    xh = jnp.concatenate([jnp.broadcast_to(xn, (32, M)) for xn in xns], axis=0).astype(BF16)
    for j in range(4):
        lhs_v[j] = xh[:, j * 128:(j + 1) * 128]

    dma(I_WQ).wait()
    q = (expand_matmul(wq_v) * (D ** -0.5)).astype(BF16)

    dma(I_WUK).wait()

    def qlat_body(j, c):
        w = wuk_v[pl.ds(pl.multiple_of(j * 4096, 4096), 4096), :]
        full = lax.dot_general(q, w, NT, preferred_element_type=F32)
        lhs_v[j] = lax.dot_general(mask_diag(full), e0_v[...], NT, preferred_element_type=F32).astype(BF16)
        return c
    lax.fori_loop(0, 4, qlat_body, 0)
    qlat = jnp.concatenate([lhs_v[j] for j in range(4)], axis=1)

    dma(I_C0).wait()
    ctxs = []
    for b in range(B):
        qb = qlat[b * 32:(b + 1) * 32]

        def flash(i, carry, b=b, qb=qb):
            m, l, acc = carry
            if b == 1:
                for k, lo in enumerate(CKV1_SPLITS[:-1]):
                    @pl.when(i == lo // KT)
                    def _():
                        dma(I_C1 + k).wait()
            c = ckv_v[b, pl.ds(pl.multiple_of(i * KT, KT), KT), :]
            s = lax.dot_general(qb, c, NT, preferred_element_type=F32)
            m_new = jnp.maximum(m, jnp.max(s, axis=-1, keepdims=True))
            alpha = jnp.exp(m - m_new)
            p = jnp.exp(s - m_new)
            l = alpha * l + jnp.sum(p, axis=-1, keepdims=True)
            acc = alpha * acc + jnp.dot(p.astype(BF16), c, preferred_element_type=F32)
            return m_new, l, acc
        m0 = jnp.full((32, 1), -jnp.inf, F32)
        m, l, acc = lax.fori_loop(0, SK // KT, flash, (m0, jnp.zeros((32, 1), F32), jnp.zeros((32, DC), F32)))
        ctxs.append(acc / l)
    ctxlat = jnp.concatenate(ctxs, axis=0).astype(BF16)
    for j in range(4):
        lhs_v[j] = ctxlat[:, j * 128:(j + 1) * 128]

    dma(I_WUV).wait()
    ctx = expand_matmul(wuv_v)
    r8 = lax.broadcasted_iota(jnp.int32, (8, 128), 0)
    for h in range(H):
        g = h // 8
        lo_v[h] = jnp.concatenate(
            [jnp.where(r8 == h % 8, ctx[b * 32 + g * 8:b * 32 + g * 8 + 8], 0.0) for b in range(B)], axis=0
        ).astype(BF16)

    dma(I_B1).wait()
    dma(I_B2).wait()
    dma(I_W1).wait()
    x16 = xh[24:40]
    hid = jnp.dot(x16, w1_v[...], preferred_element_type=F32) + b1_v[...].astype(F32).reshape(1, F)
    hid = jax.nn.gelu(hid, approximate=True).astype(BF16)
    dma(I_W2).wait()
    ff = jnp.dot(hid, w2_v[...], preferred_element_type=F32) + b2_v[...].astype(F32).reshape(1, M)
    gate = ff * jax.nn.sigmoid(ff)

    def wo_body(h, acc):
        for k, lo in enumerate(WO_SPLITS[:-1]):
            @pl.when(h == lo)
            def _():
                dma(I_WO + k).wait()
        return acc + jnp.dot(lo_v[h], wo_v[h], preferred_element_type=F32)
    s16 = lax.fori_loop(0, H, wo_body, jnp.zeros((16, M), F32))
    for b in range(B):
        sb = jnp.sum(s16[b * 8:(b + 1) * 8], axis=0, keepdims=True)
        out_v[b] = (xs[b] + sb * gate[b * 8:b * 8 + 1]).astype(BF16)
    dma(I_OUT).start()
    dma(I_OUT).wait()


@jax.jit
def pallas_recurrent_scan__compressed_kv_cla__dense_activation_gelu__decode_kernel(
    A_x: jax.Array,
    A_c_kv: jax.Array,
    A_w_q: jax.Array,
    A_w_uk: jax.Array,
    A_w_uv: jax.Array,
    A_w_o: jax.Array,
    B_x: jax.Array,
    B_w1: jax.Array,
    B_b1: jax.Array,
    B_w2: jax.Array,
    B_b2: jax.Array,
):
    del B_x
    n_sems = 4 + (len(CKV1_SPLITS) - 1) + 5 + (len(WO_SPLITS) - 1) + 1
    anyspec = pl.BlockSpec(memory_space=pl.ANY)
    return pl.pallas_call(
        _kernel,
        out_shape=jax.ShapeDtypeStruct((B, 1, M), BF16),
        in_specs=[anyspec] * 10,
        out_specs=anyspec,
        scratch_shapes=[
            pltpu.VMEM((B, 1, M), BF16),
            pltpu.VMEM((F,), BF16),
            pltpu.VMEM((M,), BF16),
            pltpu.VMEM((M * H, D), BF16),
            pltpu.VMEM((DC * H, D), BF16),
            pltpu.VMEM((DC * H, D), BF16),
            pltpu.VMEM((H, D, M), BF16),
            pltpu.VMEM((M, F), BF16),
            pltpu.VMEM((F, M), BF16),
            pltpu.VMEM((B, SK, DC), BF16),
            pltpu.VMEM((128, 4096), BF16),
            pltpu.VMEM((4, 64, 128), BF16),
            pltpu.VMEM((H, 16, 128), BF16),
            pltpu.VMEM((B, 1, M), BF16),
            pltpu.SemaphoreType.DMA((n_sems,)),
        ],
        compiler_params=pltpu.CompilerParams(vmem_limit_bytes=100 * 1024 * 1024),
    )(A_x, A_c_kv, A_w_q.reshape(M * H, D), A_w_uk.reshape(DC * H, D), A_w_uv.reshape(DC * H, D),
      A_w_o, B_w1, B_b1, B_w2, B_b2)
```

```python
import jax
import jax.numpy as jnp
from jax import lax
import jax.experimental.pallas as pl
import jax.experimental.pallas.tpu as pltpu

B, H, D, M, DC, SK, F = 2, 32, 128, 512, 512, 16384, 1792
KT = 1024
CKV1_SPLITS = (0, 8192, 12288, 14336, 16384)
WO_SPLITS = (0, 16, 24, 28, 30, 31, 32)
NT = (((1,), (1,)), ((), ()))
F32, BF16 = jnp.float32, jnp.bfloat16


def _kernel(x_hbm, ckv_hbm, wq_hbm, wuk_hbm, wuv_hbm, wo_hbm, w1_hbm, b1_hbm, w2_hbm, b2_hbm,
            o_hbm,
            x_v, b1_v, b2_v, wq_v, wuk_v, wuv_v, wo_v, w1_v, w2_v, ckv_v,
            e0_v, lhs_v, lo_v, out_v, sems):
    copies = [
        (x_hbm, x_v), (wq_hbm, wq_v), (wuk_hbm, wuk_v), (ckv_hbm.at[0], ckv_v.at[0]),
    ]
    I_X, I_WQ, I_WUK, I_C0 = range(4)
    I_C1 = len(copies)
    for lo, hi in zip(CKV1_SPLITS[:-1], CKV1_SPLITS[1:]):
        copies.append((ckv_hbm.at[1, pl.ds(lo, hi - lo)], ckv_v.at[1, pl.ds(lo, hi - lo)]))
    I_WUV = len(copies)
    copies += [(wuv_hbm, wuv_v), (b1_hbm, b1_v), (b2_hbm, b2_v), (w1_hbm, w1_v), (w2_hbm, w2_v)]
    I_B1, I_B2, I_W1, I_W2 = I_WUV + 1, I_WUV + 2, I_WUV + 3, I_WUV + 4
    I_WO = len(copies)
    for lo, hi in zip(WO_SPLITS[:-1], WO_SPLITS[1:]):
        copies.append((wo_hbm.at[pl.ds(lo * D, (hi - lo) * D)], wo_v.at[pl.ds(lo * D, (hi - lo) * D)]))
    I_OUT = len(copies)
    copies.append((out_v, o_hbm))

    def dma(i):
        return pltpu.make_async_copy(copies[i][0], copies[i][1], sems.at[i])

    for i in range(I_OUT):
        dma(i).start()

    def gen_e0(t, c):
        r = lax.broadcasted_iota(jnp.int32, (128, 128), 1) + t * 128
        m = lax.broadcasted_iota(jnp.int32, (128, 128), 0)
        e0_v[:, pl.ds(pl.multiple_of(t * 128, 128), 128)] = jnp.where((r >> 5) == m, 1.0, 0.0).astype(BF16)
        return c
    lax.fori_loop(0, 32, gen_e0, 0)

    row = lax.broadcasted_iota(jnp.int32, (64, 128), 0)
    lane = lax.broadcasted_iota(jnp.int32, (64, 128), 1)
    diag = (row & 31) == (lane & 31)

    def mask_diag(v):
        parts = [jnp.where(diag, v[:, t * 128:(t + 1) * 128], 0.0) for t in range(v.shape[1] // 128)]
        return jnp.concatenate(parts, axis=1).astype(BF16)

    def expand_matmul(w_v):
        def body(j, acc):
            xr = jnp.dot(lhs_v[j], e0_v[...], preferred_element_type=F32)
            w = w_v[pl.ds(pl.multiple_of(j * 4096, 4096), 4096), :]
            return acc + jnp.dot(mask_diag(xr), w, preferred_element_type=F32)
        return lax.fori_loop(0, 4, body, jnp.zeros((64, 128), F32))

    dma(I_X).wait()
    x = x_v[...].astype(F32)
    mu = jnp.mean(x, axis=-1, keepdims=True)
    xc = x - mu
    var = jnp.mean(xc * xc, axis=-1, keepdims=True)
    xn = xc / jnp.sqrt(var + 1e-5)
    xh = jnp.concatenate([jnp.broadcast_to(xn[b:b + 1], (32, M)) for b in range(B)], axis=0).astype(BF16)
    for j in range(4):
        lhs_v[j] = xh[:, j * 128:(j + 1) * 128]

    dma(I_WQ).wait()
    q = (expand_matmul(wq_v) * (D ** -0.5)).astype(BF16)

    dma(I_WUK).wait()

    def qlat_body(j, c):
        w = wuk_v[pl.ds(pl.multiple_of(j * 4096, 4096), 4096), :]
        full = lax.dot_general(q, w, NT, preferred_element_type=F32)
        lhs_v[j] = lax.dot_general(mask_diag(full), e0_v[...], NT, preferred_element_type=F32).astype(BF16)
        return c
    lax.fori_loop(0, 4, qlat_body, 0)
    qlat = jnp.concatenate([lhs_v[j] for j in range(4)], axis=1)

    dma(I_C0).wait()
    ctxs = []
    for b in range(B):
        qb = qlat[b * 32:(b + 1) * 32]

        def flash(i, carry, b=b, qb=qb):
            m, l, acc = carry
            if b == 1:
                for k, lo in enumerate(CKV1_SPLITS[:-1]):
                    @pl.when(i == lo // KT)
                    def _():
                        dma(I_C1 + k).wait()
            c = ckv_v[b, pl.ds(pl.multiple_of(i * KT, KT), KT), :]
            s = lax.dot_general(qb, c, NT, preferred_element_type=F32)
            m_new = jnp.maximum(m, jnp.max(s, axis=-1, keepdims=True))
            alpha = jnp.exp(m - m_new)
            p = jnp.exp(s - m_new)
            l = alpha * l + jnp.sum(p, axis=-1, keepdims=True)
            acc = alpha * acc + jnp.dot(p.astype(BF16), c, preferred_element_type=F32)
            return m_new, l, acc
        m0 = jnp.full((32, 1), -jnp.inf, F32)
        m, l, acc = lax.fori_loop(0, SK // KT, flash, (m0, jnp.zeros((32, 1), F32), jnp.zeros((32, DC), F32)))
        ctxs.append(acc / l)
    ctxlat = jnp.concatenate(ctxs, axis=0).astype(BF16)
    for j in range(4):
        lhs_v[j] = ctxlat[:, j * 128:(j + 1) * 128]

    dma(I_WUV).wait()
    ctx = expand_matmul(wuv_v)
    for h in range(H):
        lo_v[:, h * D:(h + 1) * D] = jnp.concatenate([ctx[b * H + h:b * H + h + 1] for b in range(B)], axis=0)

    dma(I_B1).wait()
    dma(I_B2).wait()
    dma(I_W1).wait()
    hid = jnp.dot(xn.astype(BF16), w1_v[...], preferred_element_type=F32) + b1_v[...].astype(F32).reshape(1, F)
    hid = jax.nn.gelu(hid, approximate=True).astype(BF16)
    dma(I_W2).wait()
    ff = jnp.dot(hid, w2_v[...], preferred_element_type=F32) + b2_v[...].astype(F32).reshape(1, M)
    gate = ff * jax.nn.sigmoid(ff)

    s = jnp.zeros((B, M), F32)
    for k, (lo, hi) in enumerate(zip(WO_SPLITS[:-1], WO_SPLITS[1:])):
        dma(I_WO + k).wait()
        s = s + jnp.dot(lo_v[:, lo * D:hi * D].astype(BF16), wo_v[lo * D:hi * D, :], preferred_element_type=F32)
    out_v[...] = (x + s * gate).astype(BF16)
    dma(I_OUT).start()
    dma(I_OUT).wait()


@jax.jit
def pallas_recurrent_scan__compressed_kv_cla__dense_activation_gelu__decode_kernel(
    A_x: jax.Array,
    A_c_kv: jax.Array,
    A_w_q: jax.Array,
    A_w_uk: jax.Array,
    A_w_uv: jax.Array,
    A_w_o: jax.Array,
    B_x: jax.Array,
    B_w1: jax.Array,
    B_b1: jax.Array,
    B_w2: jax.Array,
    B_b2: jax.Array,
):
    del B_x
    n_sems = 4 + (len(CKV1_SPLITS) - 1) + 5 + (len(WO_SPLITS) - 1) + 1
    anyspec = pl.BlockSpec(memory_space=pl.ANY)
    return pl.pallas_call(
        _kernel,
        out_shape=jax.ShapeDtypeStruct((B, M), BF16),
        in_specs=[anyspec] * 10,
        out_specs=anyspec,
        scratch_shapes=[
            pltpu.VMEM((B, M), BF16),
            pltpu.VMEM((F,), BF16),
            pltpu.VMEM((M,), BF16),
            pltpu.VMEM((M * H, D), BF16),
            pltpu.VMEM((DC * H, D), BF16),
            pltpu.VMEM((DC * H, D), BF16),
            pltpu.VMEM((H * D, M), BF16),
            pltpu.VMEM((M, F), BF16),
            pltpu.VMEM((F, M), BF16),
            pltpu.VMEM((B, SK, DC), BF16),
            pltpu.VMEM((128, 4096), BF16),
            pltpu.VMEM((4, 64, 128), BF16),
            pltpu.VMEM((B, H * D), F32),
            pltpu.VMEM((B, M), BF16),
            pltpu.SemaphoreType.DMA((n_sems,)),
        ],
        compiler_params=pltpu.CompilerParams(vmem_limit_bytes=100 * 1024 * 1024),
    )(A_x.reshape(B, M), A_c_kv, A_w_q.reshape(M * H, D), A_w_uk.reshape(DC * H, D), A_w_uv.reshape(DC * H, D),
      A_w_o.reshape(H * D, M), B_w1, B_b1, B_w2, B_b2).reshape(B, 1, M)
```

```python
import jax
import jax.numpy as jnp
from jax import lax
import jax.experimental.pallas as pl
import jax.experimental.pallas.tpu as pltpu

B, H, D, M, DC, SK, F = 2, 32, 128, 512, 512, 16384, 1792
KT = 1024
CKV_SPLITS = (0, 16384, 26624, 32768)
WO_SPLITS = (0, 20, 28, 31, 32)
G, NLOOP = 4, 7
NT = (((1,), (1,)), ((), ()))
F32, BF16 = jnp.float32, jnp.bfloat16


def _kernel(x_hbm, ckv_hbm, wq_hbm, wuk_hbm, wuv_hbm, wo_hbm, w1_hbm, b1_hbm, w2_hbm, b2_hbm,
            o_hbm,
            x_v, b1_v, b2_v, wq_v, wuk_v, wuv_v, wo_v, w1_v, w2_v, ckv_v,
            e0_v, lhs_v, lo_v, out_v, sems):
    copies = [(x_hbm, x_v), (wq_hbm, wq_v), (wuk_hbm, wuk_v)]
    I_X, I_WQ, I_WUK = range(3)
    I_C = len(copies)
    for lo, hi in zip(CKV_SPLITS[:-1], CKV_SPLITS[1:]):
        copies.append((ckv_hbm.at[pl.ds(lo, hi - lo)], ckv_v.at[pl.ds(lo, hi - lo)]))
    I_WUV = len(copies)
    copies += [(wuv_hbm, wuv_v), (b1_hbm, b1_v), (b2_hbm, b2_v), (w1_hbm, w1_v), (w2_hbm, w2_v)]
    I_B1, I_B2, I_W1, I_W2 = I_WUV + 1, I_WUV + 2, I_WUV + 3, I_WUV + 4
    I_WO = len(copies)
    for lo, hi in zip(WO_SPLITS[:-1], WO_SPLITS[1:]):
        copies.append((wo_hbm.at[pl.ds(lo * D, (hi - lo) * D)], wo_v.at[pl.ds(lo * D, (hi - lo) * D)]))
    I_OUT = len(copies)
    copies.append((out_v, o_hbm))

    sem_of = [0, 0, 0] + list(range(1, 5)) + [5, 5, 5, 5] + list(range(6, 10)) + [0]
    assert len(sem_of) == len(copies)

    def dma(i):
        return pltpu.make_async_copy(copies[i][0], copies[i][1], sems.at[sem_of[i]])

    for i in range(I_OUT):
        dma(i).start()

    def gen_e0(t, c):
        r = lax.broadcasted_iota(jnp.int32, (128, 128), 1) + t * 128
        m = lax.broadcasted_iota(jnp.int32, (128, 128), 0)
        e0_v[:, pl.ds(pl.multiple_of(t * 128, 128), 128)] = jnp.where((r >> 5) == m, 1.0, 0.0).astype(BF16)
        return c
    lax.fori_loop(0, 32, gen_e0, 0)

    row = lax.broadcasted_iota(jnp.int32, (64, 128), 0)
    lane = lax.broadcasted_iota(jnp.int32, (64, 128), 1)
    diag = (row & 31) == (lane & 31)

    def mask_diag(v):
        parts = [jnp.where(diag, v[:, t * 128:(t + 1) * 128], 0.0) for t in range(v.shape[1] // 128)]
        return jnp.concatenate(parts, axis=1).astype(BF16)

    def expand_matmul(w_v):
        def body(j, acc):
            xr = jnp.dot(lhs_v[j], e0_v[...], preferred_element_type=F32)
            w = w_v[pl.ds(pl.multiple_of(j * 4096, 4096), 4096), :]
            return acc + jnp.dot(mask_diag(xr), w, preferred_element_type=F32)
        return lax.fori_loop(0, 4, body, jnp.zeros((64, 128), F32))

    dma(I_X).wait()
    dma(I_WQ).wait()
    dma(I_WUK).wait()
    x = x_v[...].astype(F32)
    mu = jnp.mean(x, axis=-1, keepdims=True)
    xc = x - mu
    var = jnp.mean(xc * xc, axis=-1, keepdims=True)
    xn = xc / jnp.sqrt(var + 1e-5)
    xh = jnp.concatenate([jnp.broadcast_to(xn[b:b + 1], (32, M)) for b in range(B)], axis=0).astype(BF16)
    for j in range(4):
        lhs_v[j] = xh[:, j * 128:(j + 1) * 128]

    q = (expand_matmul(wq_v) * (D ** -0.5)).astype(BF16)

    def qlat_body(j, c):
        w = wuk_v[pl.ds(pl.multiple_of(j * 4096, 4096), 4096), :]
        full = lax.dot_general(q, w, NT, preferred_element_type=F32)
        lhs_v[j] = lax.dot_general(mask_diag(full), e0_v[...], NT, preferred_element_type=F32).astype(BF16)
        return c
    lax.fori_loop(0, 4, qlat_body, 0)
    qlat = jnp.concatenate([lhs_v[j] for j in range(4)], axis=1)

    ctxs = []
    for b in range(B):
        qb = qlat[b * 32:(b + 1) * 32]

        def flash(i, carry, b=b, qb=qb):
            m, l, acc = carry
            for k, lo in enumerate(CKV_SPLITS[:-1]):
                if lo // SK == b:
                    @pl.when(i == (lo % SK) // KT)
                    def _():
                        dma(I_C + k).wait()
            c = ckv_v[pl.ds(pl.multiple_of(b * SK + i * KT, KT), KT), :]
            s = lax.dot_general(qb, c, NT, preferred_element_type=F32)
            m_new = jnp.maximum(m, jnp.max(s, axis=-1, keepdims=True))
            alpha = jnp.exp(m - m_new)
            p = jnp.exp(s - m_new)
            l = alpha * l + jnp.sum(p, axis=-1, keepdims=True)
            acc = alpha * acc + jnp.dot(p.astype(BF16), c, preferred_element_type=F32)
            return m_new, l, acc
        m0 = jnp.full((32, 1), -jnp.inf, F32)
        m, l, acc = lax.fori_loop(0, SK // KT, flash, (m0, jnp.zeros((32, 1), F32), jnp.zeros((32, DC), F32)))
        ctxs.append(acc / l)
    ctxlat = jnp.concatenate(ctxs, axis=0).astype(BF16)
    for j in range(4):
        lhs_v[j] = ctxlat[:, j * 128:(j + 1) * 128]

    dma(I_WUV).wait()
    ctx = expand_matmul(wuv_v)
    r8 = lax.broadcasted_iota(jnp.int32, (8, D), 0)
    for h in range(H):
        lo_v[h // G, :, (h % G) * D:(h % G + 1) * D] = jnp.where(
            r8 == 0, ctx[h:h + 1], jnp.where(r8 == 1, ctx[H + h:H + h + 1], 0.0))

    dma(I_B1).wait()
    dma(I_B2).wait()
    dma(I_W1).wait()
    dma(I_W2).wait()
    hid = jnp.dot(xn.astype(BF16), w1_v[...], preferred_element_type=F32) + b1_v[...].astype(F32).reshape(1, F)
    hid = jax.nn.gelu(hid, approximate=True).astype(BF16)
    ff = jnp.dot(hid, w2_v[...], preferred_element_type=F32) + b2_v[...].astype(F32).reshape(1, M)
    gate = ff * jax.nn.sigmoid(ff)

    def wo_body(i, acc):
        for k, lo in enumerate(WO_SPLITS[:-1]):
            if lo < NLOOP * G:
                @pl.when(i == lo // G)
                def _():
                    dma(I_WO + k).wait()
        w = wo_v[pl.ds(pl.multiple_of(i * G * D, G * D), G * D), :]
        return acc + jnp.dot(lo_v[i].astype(BF16), w, preferred_element_type=F32)
    s = lax.fori_loop(0, NLOOP, wo_body, jnp.zeros((8, M), F32))
    for k, (lo, hi) in enumerate(zip(WO_SPLITS[:-1], WO_SPLITS[1:])):
        if lo >= NLOOP * G:
            dma(I_WO + k).wait()
            lhs = jnp.concatenate([lo_v[h // G, :, (h % G) * D:(h % G + 1) * D] for h in range(lo, hi)], axis=1)
            s = s + jnp.dot(lhs.astype(BF16), wo_v[lo * D:hi * D, :], preferred_element_type=F32)
    out_v[...] = (x + s[0:B] * gate).astype(BF16)
    dma(I_OUT).start()
    dma(I_OUT).wait()


@jax.jit
def pallas_recurrent_scan__compressed_kv_cla__dense_activation_gelu__decode_kernel(
    A_x: jax.Array,
    A_c_kv: jax.Array,
    A_w_q: jax.Array,
    A_w_uk: jax.Array,
    A_w_uv: jax.Array,
    A_w_o: jax.Array,
    B_x: jax.Array,
    B_w1: jax.Array,
    B_b1: jax.Array,
    B_w2: jax.Array,
    B_b2: jax.Array,
):
    del B_x
    n_sems = 10
    anyspec = pl.BlockSpec(memory_space=pl.ANY)
    return pl.pallas_call(
        _kernel,
        out_shape=jax.ShapeDtypeStruct((B, M), BF16),
        in_specs=[anyspec] * 10,
        out_specs=anyspec,
        scratch_shapes=[
            pltpu.VMEM((B, M), BF16),
            pltpu.VMEM((F,), BF16),
            pltpu.VMEM((M,), BF16),
            pltpu.VMEM((M * H, D), BF16),
            pltpu.VMEM((DC * H, D), BF16),
            pltpu.VMEM((DC * H, D), BF16),
            pltpu.VMEM((H * D, M), BF16),
            pltpu.VMEM((M, F), BF16),
            pltpu.VMEM((F, M), BF16),
            pltpu.VMEM((B * SK, DC), BF16),
            pltpu.VMEM((128, 4096), BF16),
            pltpu.VMEM((4, 64, 128), BF16),
            pltpu.VMEM((H // G, 8, G * D), F32),
            pltpu.VMEM((B, M), BF16),
            pltpu.SemaphoreType.DMA((n_sems,)),
        ],
        compiler_params=pltpu.CompilerParams(vmem_limit_bytes=100 * 1024 * 1024),
    )(A_x.reshape(B, M), A_c_kv.reshape(B * SK, DC), A_w_q.reshape(M * H, D), A_w_uk.reshape(DC * H, D), A_w_uv.reshape(DC * H, D),
      A_w_o.reshape(H * D, M), B_w1, B_b1, B_w2, B_b2).reshape(B, 1, M)
```
